```python
import os as _os
_os.environ.setdefault("JAX_PLATFORMS", "cpu")
import jax
import jax.numpy as jnp

def _softmax(x, axis=-1):
    return jax.nn.softmax(x, axis=axis)
def _gelu(x):
    return jax.nn.gelu(x, approximate=True)
def _silu(x):
    return jax.nn.silu(x)
def _sigmoid(x):
    return jax.nn.sigmoid(x)
def _layernorm(x, axis=-1, eps=1e-5):
    m = jnp.mean(x, axis=axis, keepdims=True)
    v = jnp.var(x, axis=axis, keepdims=True)
    return (x - m) / jnp.sqrt(v + eps)
def _scatter_add(tgt, idx, src, axis=0):
    return tgt.at[idx].add(src)
def _segment_sum(src, seg, n):
    return jax.ops.segment_sum(src, seg, n)
class _Rng:
    def __init__(self, key):
        self._k = key
    def _next(self):
        self._k, sub = jax.random.split(self._k)
        return sub
    def normal(self, shape):
        return jax.random.normal(self._next(), shape, dtype=jnp.bfloat16)
    def randint(self, lo, hi, shape):
        return jax.random.randint(self._next(), shape, lo, hi, dtype=jnp.int32)
    def uniform(self, shape, lo=0.0, hi=1.0):
        return jax.random.uniform(self._next(), shape, jnp.bfloat16, lo, hi)
    def permutation(self, n):
        return jax.random.permutation(self._next(), n)


kernel_name = 'gated_mix__gqa_block_cached__dense_activation_squared_relu__decode'

def setup_inputs():
    _rng = _Rng(jax.random.key(int.from_bytes(__import__("os").urandom(4), "little")))
    _w = (lambda a: (lambda t: t.astype(jnp.bfloat16) if jnp.issubdtype(t.dtype, jnp.floating) else t)(jnp.asarray(a)))
    def _A_setup():
        B, Sq, D = 4, 1, 512
        Hq, Hkv, Sk, Dh = 32, 8, 4096, 128
        assert Hq % Hkv == 0, (Hq, Hkv)
        return {
            "x": _w((lambda *s: _rng.normal(s) * 0.05)(B, Sq, D)),
            "k_cache": _w((lambda *s: _rng.normal(s) * 3.2)(B, Hkv, Sk, Dh)),
            "v_cache": _w((lambda *s: _rng.normal(s) * 1.6)(B, Hkv, Sk, Dh)),
            "wq": _w((lambda *s: _rng.normal(s) * 3.2)(D, Hq * Dh) * (D ** -0.5)),
            "wo": _w((lambda *s: _rng.normal(s) * 1.6)(Hq * Dh, D) * ((Hq * Dh) ** -0.5)),
        }
    _A_in = _A_setup()

    def _B_setup():
        B, S, D, F = 4, 1, 512, 1792
        return {
            "x": _w((lambda *s: _rng.normal(s) * 0.05)(B, S, D)),
            "w1": _w((lambda *s: _rng.normal(s) * 0.1)(D, F)),
            "b1": _w((lambda *s: _rng.normal(s) * 0.05)(F)),
            "w2": _w((lambda *s: _rng.normal(s) * 0.05)(F, D)),
            "b2": _w((lambda *s: _rng.normal(s) * 0.05)(D)),
        }
    _B_in = _B_setup()

    return {
        "A_x": _A_in["x"],
        "A_k_cache": _A_in["k_cache"],
        "A_v_cache": _A_in["v_cache"],
        "A_wq": _A_in["wq"],
        "A_wo": _A_in["wo"],
        "B_x": _B_in["x"],
        "B_w1": _B_in["w1"],
        "B_b1": _B_in["b1"],
        "B_w2": _B_in["w2"],
        "B_b2": _B_in["b2"],
        "gate_w": _w((lambda *s: _rng.normal(s) * 0.05)(512) * 16.0),
    }

def reference(A_x, A_k_cache, A_v_cache, A_wq, A_wo, B_x, B_w1, B_b1, B_w2, B_b2, gate_w):
    def _A_ref(x, k_cache, v_cache, wq, wo):
        B, Sq, D = x.shape
        Hq, Dh = 32, 128
        Hkv = k_cache.shape[1]
        rep = Hq // Hkv
        q = (lambda x, *d: x.transpose(*d))((x @ wq).reshape(B, Sq, Hq, Dh), 0, 2, 1, 3)
        k = jnp.repeat(k_cache, rep, axis=1)
        v = jnp.repeat(v_cache, rep, axis=1)
        scores = jnp.einsum("bhqd,bhkd->bhqk", q, k) * (Dh ** -0.5)
        p = _softmax(scores, axis=-1)
        o = jnp.einsum("bhqk,bhkd->bhqd", p, v)
        return (lambda x, *d: x.transpose(*d))(o, 0, 2, 1, 3).reshape(B, Sq, Hq * Dh) @ wo

    def _B_ref(x, w1, b1, w2, b2):
        h = jnp.einsum("bsd,df->bsf", x, w1) + b1
        zero = jnp.zeros_like(h)
        r = jnp.where(h > zero, h, zero)
        h = r * r
        out = jnp.einsum("bsf,fd->bsd", h, w2) + b2
        return out

    x = A_x
    g = _sigmoid((x * gate_w).sum(-1, keepdims=True))
    a = _A_ref(x, A_k_cache, A_v_cache, A_wq, A_wo)
    b = _B_ref(x, B_w1, B_b1, B_w2, B_b2)
    return g * a + (1 - g) * b
```

```python
import jax
import jax.numpy as jnp
from jax import lax
import jax.experimental.pallas as pl
import jax.experimental.pallas.tpu as pltpu

B = 4
D = 512
HQ = 32
HKV = 8
REP = HQ // HKV
SK = 4096
DH = 128
F = 1792
SCALE = DH ** -0.5

_HBM = pltpu.MemorySpace.HBM
_NT = (((1,), (1,)), ((), ()))


def _kernel(x_hbm, k_hbm, v_hbm, wq_hbm, wo_hbm, w1_hbm, b1_hbm, w2_hbm, b2_hbm, gw_hbm,
            o_ref,
            x_s, gw_s, b1_s, b2_s, wq_s, wo_s, w1_s, w2_s, kbuf, vbuf, q_s, o_s,
            small_sem, w_sem, k_sem, v_sem):
    small = [
        pltpu.make_async_copy(x_hbm, x_s, small_sem.at[0]),
        pltpu.make_async_copy(gw_hbm, gw_s, small_sem.at[1]),
        pltpu.make_async_copy(b1_hbm, b1_s, small_sem.at[2]),
        pltpu.make_async_copy(b2_hbm, b2_s, small_sem.at[3]),
    ]
    HD = D // 2
    wq_c = [pltpu.make_async_copy(wq_hbm.at[pl.ds(i * HD, HD)], wq_s.at[pl.ds(i * HD, HD)], w_sem.at[i])
            for i in range(2)]
    w1_c = pltpu.make_async_copy(w1_hbm, w1_s, w_sem.at[2])
    w2_c = pltpu.make_async_copy(w2_hbm, w2_s, w_sem.at[3])
    HO = HQ * DH // 2
    wo_c = [pltpu.make_async_copy(wo_hbm.at[pl.ds(i * HO, HO)], wo_s.at[pl.ds(i * HO, HO)], w_sem.at[4 + i])
            for i in range(2)]

    def k_copy(g, b):
        return pltpu.make_async_copy(k_hbm.at[b, g], kbuf.at[b], k_sem.at[b])

    def v_copy(g, b):
        return pltpu.make_async_copy(v_hbm.at[b, g], vbuf.at[b], v_sem.at[b])

    wq_c[0].start()
    for c in small:
        c.start()
    wq_c[1].start()

    small[0].wait()
    xb = x_s[...]

    wq_c[0].wait()
    w1_c.start()
    q = jnp.dot(xb[:, :HD], wq_s[0:HD, :], preferred_element_type=jnp.float32)
    wq_c[1].wait()
    w2_c.start()
    q = q + jnp.dot(xb[:, HD:], wq_s[HD:D, :], preferred_element_type=jnp.float32)
    for h in range(HQ):
        q_s[h * 8:h * 8 + B, :] = q[:, h * DH:(h + 1) * DH]

    small[2].wait()
    w1_c.wait()
    wo_c[0].start()
    h1 = jnp.dot(xb, w1_s[...], preferred_element_type=jnp.float32)
    h1 = h1 + b1_s[...].astype(jnp.float32).reshape(1, F)
    r = jnp.maximum(h1, 0.0)
    hsq = (r * r).astype(jnp.bfloat16)
    small[3].wait()
    w2_c.wait()
    wo_c[1].start()
    ffn = jnp.dot(hsq, w2_s[...], preferred_element_type=jnp.float32)
    ffn = ffn + b2_s[...].astype(jnp.float32).reshape(1, D)

    small[1].wait()
    xg = xb.astype(jnp.float32) * gw_s[...].astype(jnp.float32).reshape(1, D)
    gate = jax.nn.sigmoid(jnp.sum(xg, axis=-1, keepdims=True))

    wo_c[0].wait()
    k_copy(0, 0).start()
    v_copy(0, 0).start()
    wo_c[1].wait()
    for b in range(1, B):
        k_copy(0, b).start()
        v_copy(0, b).start()

    def group(g, acc):
        for b in range(B):
            k_copy(g, b).wait()
            qv = q_s[pl.ds(g * (REP * 8) + b, REP, stride=8), :].astype(jnp.bfloat16)
            s = lax.dot_general(qv, kbuf[b], _NT, preferred_element_type=jnp.float32) * SCALE

            @pl.when(g + 1 < HKV)
            def _():
                k_copy(g + 1, b).start()

            m = jnp.max(s, axis=-1, keepdims=True)
            p = jnp.exp(s - m)
            l = jnp.sum(p, axis=-1, keepdims=True)
            v_copy(g, b).wait()
            o = jnp.dot(p.astype(jnp.bfloat16), vbuf[b], preferred_element_type=jnp.float32)

            @pl.when(g + 1 < HKV)
            def _():
                v_copy(g + 1, b).start()

            o_s[pl.ds(b, REP, stride=8), :] = o / l
        lhs = jnp.concatenate([o_s[j * 8:j * 8 + B, :] for j in range(REP)], axis=1).astype(jnp.bfloat16)
        wo_g = wo_s[pl.ds(pl.multiple_of(g * (REP * DH), REP * DH), REP * DH), :]
        return acc + jnp.dot(lhs, wo_g, preferred_element_type=jnp.float32)

    attn = lax.fori_loop(0, HKV, group, jnp.zeros((B, D), jnp.float32))

    o_ref[...] = (gate * attn + (1.0 - gate) * ffn).astype(o_ref.dtype)


@jax.jit
def pallas_gated_mix__gqa_block_cached__dense_activation_squared_relu__decode_kernel(
    A_x: jax.Array,
    A_k_cache: jax.Array,
    A_v_cache: jax.Array,
    A_wq: jax.Array,
    A_wo: jax.Array,
    B_x: jax.Array,
    B_w1: jax.Array,
    B_b1: jax.Array,
    B_w2: jax.Array,
    B_b2: jax.Array,
    gate_w: jax.Array,
):
    bf16 = jnp.bfloat16
    out = pl.pallas_call(
        _kernel,
        out_shape=jax.ShapeDtypeStruct((B, D), bf16),
        in_specs=[pl.BlockSpec(memory_space=_HBM)] * 10,
        out_specs=pl.BlockSpec(memory_space=pltpu.VMEM),
        scratch_shapes=[
            pltpu.VMEM((B, D), bf16),
            pltpu.VMEM((D,), bf16),
            pltpu.VMEM((F,), bf16),
            pltpu.VMEM((D,), bf16),
            pltpu.VMEM((D, HQ * DH), bf16),
            pltpu.VMEM((HQ * DH, D), bf16),
            pltpu.VMEM((D, F), bf16),
            pltpu.VMEM((F, D), bf16),
            pltpu.VMEM((B, SK, DH), bf16),
            pltpu.VMEM((B, SK, DH), bf16),
            pltpu.VMEM((HQ * 8, DH), jnp.float32),
            pltpu.VMEM((REP * 8, DH), jnp.float32),
            pltpu.SemaphoreType.DMA((4,)),
            pltpu.SemaphoreType.DMA((6,)),
            pltpu.SemaphoreType.DMA((B,)),
            pltpu.SemaphoreType.DMA((B,)),
        ],
        compiler_params=pltpu.CompilerParams(vmem_limit_bytes=64 * 1024 * 1024),
    )(A_x.reshape(B, D), A_k_cache, A_v_cache, A_wq, A_wo, B_w1, B_b1, B_w2, B_b2, gate_w)
    return out.reshape(B, 1, D)
```

```python
import jax
import jax.numpy as jnp
from jax import lax
import jax.experimental.pallas as pl
import jax.experimental.pallas.tpu as pltpu

B = 4
D = 512
HQ = 32
HKV = 8
REP = HQ // HKV
SK = 4096
DH = 128
F = 1792
SCALE = DH ** -0.5

KV_ROWS = 128
KV_PIECES = SK // KV_ROWS
WO_PHASES = 4
LOOKAHEAD = 3

_HBM = pltpu.MemorySpace.HBM
_NT = (((1,), (1,)), ((), ()))


def _start_interleaved(n, piece0, piece1, unroll=1):
    def body(i, carry):
        piece0(i).start(priority=0)
        piece1(i).start(priority=1)
        return carry
    lax.fori_loop(0, n, body, 0, unroll=unroll)


def _kernel(x_hbm, k_hbm, v_hbm, wq_hbm, wo_hbm, w1_hbm, b1_hbm, w2_hbm, b2_hbm, gw_hbm,
            o_ref,
            x_s, gw_s, b1_s, b2_s, wq_s, wo_s, w1_s, w2_s, kv_s, q_s, o_s,
            small_sem, w_sem, wo_sem, kv_sem):
    small = [
        pltpu.make_async_copy(x_hbm, x_s, small_sem.at[0]),
        pltpu.make_async_copy(gw_hbm, gw_s, small_sem.at[1]),
        pltpu.make_async_copy(b1_hbm, b1_s, small_sem.at[2]),
        pltpu.make_async_copy(b2_hbm, b2_s, small_sem.at[3]),
    ]

    def wq_piece(half):
        def f(i):
            r = pl.multiple_of(half * (D // 2) + (i // 4) * 16, 16)
            c = pl.multiple_of((i % 4) * 1024, 1024)
            idx = (pl.ds(r, 16), pl.ds(c, 1024))
            return pltpu.make_async_copy(wq_hbm.at[idx], wq_s.at[idx], w_sem.at[0])
        return f

    def w1_piece(i):
        r = pl.multiple_of((i // 2) * 16, 16)
        c = pl.multiple_of((i % 2) * (F // 2), F // 2)
        idx = (pl.ds(r, 16), pl.ds(c, F // 2))
        return pltpu.make_async_copy(w1_hbm.at[idx], w1_s.at[idx], w_sem.at[1])

    def w2_piece(i):
        idx = pl.ds(pl.multiple_of(i * 32, 32), 32)
        return pltpu.make_async_copy(w2_hbm.at[idx], w2_s.at[idx], w_sem.at[2])

    WO_N = HQ * DH // 2 // 32 // WO_PHASES

    def wo_piece(phase, half):
        def f(i):
            r = half * (HQ * DH // 2) + (phase * WO_N + i) * 32
            idx = pl.ds(pl.multiple_of(r, 32), 32)
            return pltpu.make_async_copy(wo_hbm.at[idx], wo_s.at[idx], wo_sem.at[phase])
        return f

    def start_wo(phase):
        _start_interleaved(WO_N, wo_piece(phase, 0), wo_piece(phase, 1))

    def wait_wo(phase):
        rows = pl.ds(0, WO_N * 32)
        for _ in range(2):
            pltpu.make_async_copy(wo_s.at[rows], wo_s.at[rows], wo_sem.at[phase]).wait()

    def start_kv(g, b):
        def k_piece(i):
            idx = pl.ds(pl.multiple_of(i * KV_ROWS, KV_ROWS), KV_ROWS)
            return pltpu.make_async_copy(k_hbm.at[b, g, idx], kv_s.at[b, 0, idx], kv_sem.at[b])

        def v_piece(i):
            idx = pl.ds(pl.multiple_of(i * KV_ROWS, KV_ROWS), KV_ROWS)
            return pltpu.make_async_copy(v_hbm.at[b, g, idx], kv_s.at[b, 1, idx], kv_sem.at[b])
        _start_interleaved(KV_PIECES, k_piece, v_piece)

    def wait_kv(b):
        pltpu.make_async_copy(kv_s.at[b], kv_s.at[b], kv_sem.at[b]).wait()

    small[0].start()
    _start_interleaved(64, wq_piece(0), wq_piece(1))
    for c in small[1:]:
        c.start()
    _start_interleaved(56, w1_piece, w2_piece)
    _start_interleaved(4, lambda i: w1_piece(56 + 2 * i), lambda i: w1_piece(57 + 2 * i))
    for j in range(LOOKAHEAD):
        start_kv(j // B, j % B)

    small[0].wait()
    xb = x_s[...]
    pltpu.make_async_copy(wq_s, wq_s, w_sem.at[0]).wait()
    q = jnp.dot(xb, wq_s[...], preferred_element_type=jnp.float32)
    for h in range(HQ):
        q_s[h * 8:h * 8 + B, :] = q[:, h * DH:(h + 1) * DH]

    small[2].wait()
    pltpu.make_async_copy(w1_s, w1_s, w_sem.at[1]).wait()
    h1 = jnp.dot(xb, w1_s[...], preferred_element_type=jnp.float32)
    h1 = h1 + b1_s[...].astype(jnp.float32).reshape(1, F)
    r = jnp.maximum(h1, 0.0)
    hsq = (r * r).astype(jnp.bfloat16)
    small[3].wait()
    pltpu.make_async_copy(w2_s, w2_s, w_sem.at[2]).wait()
    ffn = jnp.dot(hsq, w2_s[...], preferred_element_type=jnp.float32)
    ffn = ffn + b2_s[...].astype(jnp.float32).reshape(1, D)

    small[1].wait()
    xg = xb.astype(jnp.float32) * gw_s[...].astype(jnp.float32).reshape(1, D)
    gate = jax.nn.sigmoid(jnp.sum(xg, axis=-1, keepdims=True))
    ffn_part = (1.0 - gate) * ffn

    def group(g, carry):
        for b in range(B):
            wait_kv(b)
            nb = (b + LOOKAHEAD) % B
            ng = g + (b + LOOKAHEAD) // B

            @pl.when(ng < HKV)
            def _():
                start_kv(ng, nb)

            if b + LOOKAHEAD >= B:
                @pl.when(ng == HKV)
                def _():
                    n0 = b + LOOKAHEAD - B
                    for ph in range(WO_PHASES):
                        if ph * LOOKAHEAD // WO_PHASES == n0:
                            start_wo(ph)

            qv = q_s[pl.ds(g * (REP * 8) + b, REP, stride=8), :].astype(jnp.bfloat16)
            s = lax.dot_general(qv, kv_s[b, 0], _NT, preferred_element_type=jnp.float32) * SCALE
            m = jnp.max(s, axis=-1, keepdims=True)
            p = jnp.exp(s - m)
            l = jnp.sum(p, axis=-1, keepdims=True)
            o = jnp.dot(p.astype(jnp.bfloat16), kv_s[b, 1], preferred_element_type=jnp.float32)
            o_s[pl.ds(g * (REP * 8) + b, REP, stride=8), :] = o / l
        return carry

    lax.fori_loop(0, HKV, group, 0)

    attn = None
    heads = WO_N * 32 // DH
    for ph in range(WO_PHASES):
        wait_wo(ph)
        for half in range(2):
            h0 = half * (HQ // 2) + ph * heads
            lhs = jnp.concatenate(
                [o_s[(h0 + j) * 8:(h0 + j) * 8 + B, :] for j in range(heads)], axis=1).astype(jnp.bfloat16)
            part = jnp.dot(lhs, wo_s[h0 * DH:(h0 + heads) * DH, :], preferred_element_type=jnp.float32)
            attn = part if attn is None else attn + part

    o_ref[...] = (gate * attn + ffn_part).astype(o_ref.dtype)


@jax.jit
def pallas_gated_mix__gqa_block_cached__dense_activation_squared_relu__decode_kernel(
    A_x: jax.Array,
    A_k_cache: jax.Array,
    A_v_cache: jax.Array,
    A_wq: jax.Array,
    A_wo: jax.Array,
    B_x: jax.Array,
    B_w1: jax.Array,
    B_b1: jax.Array,
    B_w2: jax.Array,
    B_b2: jax.Array,
    gate_w: jax.Array,
):
    bf16 = jnp.bfloat16
    out = pl.pallas_call(
        _kernel,
        out_shape=jax.ShapeDtypeStruct((B, D), bf16),
        in_specs=[pl.BlockSpec(memory_space=_HBM)] * 10,
        out_specs=pl.BlockSpec(memory_space=pltpu.VMEM),
        scratch_shapes=[
            pltpu.VMEM((B, D), bf16),
            pltpu.VMEM((D,), bf16),
            pltpu.VMEM((F,), bf16),
            pltpu.VMEM((D,), bf16),
            pltpu.VMEM((D, HQ * DH), bf16),
            pltpu.VMEM((HQ * DH, D), bf16),
            pltpu.VMEM((D, F), bf16),
            pltpu.VMEM((F, D), bf16),
            pltpu.VMEM((B, 2, SK, DH), bf16),
            pltpu.VMEM((HQ * 8, DH), jnp.float32),
            pltpu.VMEM((HQ * 8, DH), jnp.float32),
            pltpu.SemaphoreType.DMA((4,)),
            pltpu.SemaphoreType.DMA((3,)),
            pltpu.SemaphoreType.DMA((WO_PHASES,)),
            pltpu.SemaphoreType.DMA((B,)),
        ],
        compiler_params=pltpu.CompilerParams(
            vmem_limit_bytes=64 * 1024 * 1024,
            disable_bounds_checks=True,
        ),
    )(A_x.reshape(B, D), A_k_cache, A_v_cache, A_wq, A_wo, B_w1, B_b1, B_w2, B_b2, gate_w)
    return out.reshape(B, 1, D)
```

```python
import jax
import jax.numpy as jnp
from jax import lax
import jax.experimental.pallas as pl
import jax.experimental.pallas.tpu as pltpu

B = 4
D = 512
HQ = 32
HKV = 8
REP = HQ // HKV
SK = 4096
DH = 128
F = 1792
SCALE = DH ** -0.5

KV_ROWS = 128
KV_PIECES = SK // KV_ROWS
K_PARTS = 4
NSLOT = 2

WO_PHASES = (
    tuple((8 * s, 4) for s in range(4)),
    tuple((8 * s + 4, 2) for s in range(4)),
    tuple((8 * s + 6, 1) for s in range(4)),
    tuple((8 * s + 7, 1) for s in range(4)),
)

_HBM = pltpu.MemorySpace.HBM
_NT = (((1,), (1,)), ((), ()))


def _loop(n, body):
    def step(i, carry):
        body(i)
        return carry
    lax.fori_loop(0, n, step, 0)


def _wait_all(buf, sem):
    pltpu.make_async_copy(buf, buf, sem).wait()


def _kernel(x_hbm, k_hbm, v_hbm, wq_hbm, wo_hbm, w1_hbm, b1_hbm, w2_hbm, b2_hbm, gw_hbm,
            o_ref,
            x_s, gw_s, b1_s, b2_s, wq_s, wo_s, w1_s, w2_s, kv_s, q_s, o_s,
            small_sem, w_sem, wo_sem, kv_sem):
    small = [
        pltpu.make_async_copy(x_hbm, x_s, small_sem.at[0]),
        pltpu.make_async_copy(gw_hbm, gw_s, small_sem.at[1]),
        pltpu.make_async_copy(b1_hbm, b1_s, small_sem.at[2]),
        pltpu.make_async_copy(b2_hbm, b2_s, small_sem.at[3]),
    ]

    def start_wq():
        def body(i):
            for s in range(4):
                p = s * 32 + i
                idx = (pl.ds(pl.multiple_of((p // 4) * 16, 16), 16),
                       pl.ds(pl.multiple_of((p % 4) * 1024, 1024), 1024))
                pltpu.make_async_copy(wq_hbm.at[idx], wq_s.at[idx], w_sem.at[0]).start(priority=s % 2)
        _loop(32, body)

    def w1_piece(p):
        idx = (pl.ds(pl.multiple_of((p // 2) * 16, 16), 16),
               pl.ds(pl.multiple_of((p % 2) * (F // 2), F // 2), F // 2))
        return pltpu.make_async_copy(w1_hbm.at[idx], w1_s.at[idx], w_sem.at[1])

    def w2_piece(p):
        idx = pl.ds(pl.multiple_of(p * 32, 32), 32)
        return pltpu.make_async_copy(w2_hbm.at[idx], w2_s.at[idx], w_sem.at[2])

    def start_ffn(half):
        def body(i):
            p = half * 14 + i
            w1_piece(p).start(priority=0)
            w2_piece(p).start(priority=1)
            w1_piece(32 + p).start(priority=0)
            w2_piece(28 + p).start(priority=1)
        _loop(14, body)
        if half == 1:
            def rest(i):
                w1_piece(28 + i).start(priority=0)
                w1_piece(60 + i).start(priority=1)
            _loop(4, rest)

    wo_base = [0]
    for runs in WO_PHASES:
        wo_base.append(wo_base[-1] + sum(n for _, n in runs) * DH)

    def start_wo(ph):
        runs = WO_PHASES[ph]
        rows = runs[0][1] * DH

        def body(i):
            for u, (h0, _) in enumerate(runs):
                src = pl.ds(pl.multiple_of(h0 * DH + i * 32, 32), 32)
                dst = pl.ds(pl.multiple_of(wo_base[ph] + u * rows + i * 32, 32), 32)
                pltpu.make_async_copy(wo_hbm.at[src], wo_s.at[dst], wo_sem.at[ph]).start(priority=u % 2)
        _loop(rows // 32, body)

    def start_kv(g, part):
        slot = g % NSLOT
        n = KV_PIECES // K_PARTS

        def body(i):
            idx = pl.ds(pl.multiple_of((part * n + i) * KV_ROWS, KV_ROWS), KV_ROWS)
            for b in range(B):
                pltpu.make_async_copy(k_hbm.at[b, g, idx], kv_s.at[slot, b, 0, idx],
                                      kv_sem.at[slot]).start(priority=0)
                pltpu.make_async_copy(v_hbm.at[b, g, idx], kv_s.at[slot, b, 1, idx],
                                      kv_sem.at[slot]).start(priority=1)
        _loop(n, body)

    def start_next(g, part):
        @pl.when(g + 1 < HKV)
        def _():
            start_kv(g + 1, part)

        @pl.when(g + 1 == HKV)
        def _():
            if part < 2:
                start_ffn(part)
            else:
                start_wo(part - 2)

    small[0].start()
    start_wq()
    for c in small[1:]:
        c.start()
    start_kv(0, 0)

    small[0].wait()
    xb = x_s[...]
    _wait_all(wq_s, w_sem.at[0])
    start_kv(0, 1)
    q = jnp.dot(xb, wq_s[...], preferred_element_type=jnp.float32)
    start_kv(0, 2)
    for h in range(HQ):
        q_s[h * 8:h * 8 + B, :] = q[:, h * DH:(h + 1) * DH]
    start_kv(0, 3)

    def attend(g, slot, b):
        rows = pl.ds(g * (REP * 8) + b, REP, stride=8)
        qv = q_s[rows, :].astype(jnp.bfloat16)
        s = lax.dot_general(qv, kv_s[slot, b, 0], _NT, preferred_element_type=jnp.float32) * SCALE
        m = jnp.max(s, axis=-1, keepdims=True)
        p = jnp.exp(s - m)
        l = jnp.sum(p, axis=-1, keepdims=True)
        o = jnp.dot(p.astype(jnp.bfloat16), kv_s[slot, b, 1], preferred_element_type=jnp.float32)
        o_s[rows, :] = o / l

    def group(g):
        slot = g % NSLOT
        start_next(g, 0)
        start_next(g, 1)
        _wait_all(kv_s.at[slot], kv_sem.at[slot])
        attend(g, slot, 0)
        start_next(g, 2)
        attend(g, slot, 1)
        start_next(g, 3)
        attend(g, slot, 2)
        attend(g, slot, 3)

    _loop(HKV, group)

    start_wo(2)
    small[2].wait()
    _wait_all(w1_s, w_sem.at[1])
    h1 = jnp.dot(xb, w1_s[...], preferred_element_type=jnp.float32)
    h1 = h1 + b1_s[...].astype(jnp.float32).reshape(1, F)
    r = jnp.maximum(h1, 0.0)
    hsq = (r * r).astype(jnp.bfloat16)
    small[3].wait()
    _wait_all(w2_s, w_sem.at[2])
    ffn = jnp.dot(hsq, w2_s[...], preferred_element_type=jnp.float32)
    ffn = ffn + b2_s[...].astype(jnp.float32).reshape(1, D)

    small[1].wait()
    xg = xb.astype(jnp.float32) * gw_s[...].astype(jnp.float32).reshape(1, D)
    gate = jax.nn.sigmoid(jnp.sum(xg, axis=-1, keepdims=True))
    ffn_part = (1.0 - gate) * ffn

    start_wo(3)
    attn = None
    for ph, runs in enumerate(WO_PHASES):
        _wait_all(wo_s.at[pl.ds(wo_base[ph], wo_base[ph + 1] - wo_base[ph])], wo_sem.at[ph])
        for u, (h0, n) in enumerate(runs):
            lhs = jnp.concatenate(
                [o_s[(h0 + j) * 8:(h0 + j) * 8 + B, :] for j in range(n)], axis=1).astype(jnp.bfloat16)
            r0 = wo_base[ph] + u * n * DH
            part = jnp.dot(lhs, wo_s[r0:r0 + n * DH, :], preferred_element_type=jnp.float32)
            attn = part if attn is None else attn + part

    o_ref[...] = (gate * attn + ffn_part).astype(o_ref.dtype)


@jax.jit
def pallas_gated_mix__gqa_block_cached__dense_activation_squared_relu__decode_kernel(
    A_x: jax.Array,
    A_k_cache: jax.Array,
    A_v_cache: jax.Array,
    A_wq: jax.Array,
    A_wo: jax.Array,
    B_x: jax.Array,
    B_w1: jax.Array,
    B_b1: jax.Array,
    B_w2: jax.Array,
    B_b2: jax.Array,
    gate_w: jax.Array,
):
    bf16 = jnp.bfloat16
    out = pl.pallas_call(
        _kernel,
        out_shape=jax.ShapeDtypeStruct((B, D), bf16),
        in_specs=[pl.BlockSpec(memory_space=_HBM)] * 10,
        out_specs=pl.BlockSpec(memory_space=pltpu.VMEM),
        scratch_shapes=[
            pltpu.VMEM((B, D), bf16),
            pltpu.VMEM((D,), bf16),
            pltpu.VMEM((F,), bf16),
            pltpu.VMEM((D,), bf16),
            pltpu.VMEM((D, HQ * DH), bf16),
            pltpu.VMEM((HQ * DH, D), bf16),
            pltpu.VMEM((D, F), bf16),
            pltpu.VMEM((F, D), bf16),
            pltpu.VMEM((NSLOT, B, 2, SK, DH), bf16),
            pltpu.VMEM((HQ * 8, DH), jnp.float32),
            pltpu.VMEM((HQ * 8, DH), jnp.float32),
            pltpu.SemaphoreType.DMA((4,)),
            pltpu.SemaphoreType.DMA((3,)),
            pltpu.SemaphoreType.DMA((len(WO_PHASES),)),
            pltpu.SemaphoreType.DMA((NSLOT,)),
        ],
        compiler_params=pltpu.CompilerParams(vmem_limit_bytes=64 * 1024 * 1024),
    )(A_x.reshape(B, D), A_k_cache, A_v_cache, A_wq, A_wo, B_w1, B_b1, B_w2, B_b2, gate_w)
    return out.reshape(B, 1, D)
```

```python
import jax
import jax.numpy as jnp
from jax import lax
import jax.experimental.pallas as pl
import jax.experimental.pallas.tpu as pltpu

B = 4
D = 512
HQ = 32
HKV = 8
REP = HQ // HKV
SK = 4096
DH = 128
F = 1792
SCALE = DH ** -0.5

KV_ROWS = 128
KV_PIECES = SK // KV_ROWS
K_PARTS = 4
NSLOT = 2

WO_PHASES = (
    tuple((4 * s, 2) for s in range(8)),
    tuple((4 * s + 2, 1) for s in range(8)),
    tuple((8 * s + 3, 1) for s in range(4)),
    tuple((8 * s + 7, 1) for s in range(4)),
)

_HBM = pltpu.MemorySpace.HBM
_NT = (((1,), (1,)), ((), ()))


def _loop(n, body):
    def step(i, carry):
        body(i)
        return carry
    lax.fori_loop(0, n, step, 0)


def _wait_all(buf, sem):
    pltpu.make_async_copy(buf, buf, sem).wait()


def _kernel(x_hbm, k_hbm, v_hbm, wq_hbm, wo_hbm, w1_hbm, b1_hbm, w2_hbm, b2_hbm, gw_hbm,
            o_ref,
            x_s, gw_s, b1_s, b2_s, wq_s, wo_s, w1_s, w2_s, kv_s, q_s, o_s,
            small_sem, w_sem, wo_sem, kv_sem):
    small = [
        pltpu.make_async_copy(x_hbm, x_s, small_sem.at[0]),
        pltpu.make_async_copy(gw_hbm, gw_s, small_sem.at[1]),
        pltpu.make_async_copy(b1_hbm, b1_s, small_sem.at[2]),
        pltpu.make_async_copy(b2_hbm, b2_s, small_sem.at[3]),
    ]

    def start_wq():
        def body(i):
            for s in range(4):
                p = s * 32 + i
                idx = (pl.ds(pl.multiple_of((p // 2) * 8, 8), 8),
                       pl.ds(pl.multiple_of((p % 2) * 2048, 2048), 2048))
                pltpu.make_async_copy(wq_hbm.at[idx], wq_s.at[idx], w_sem.at[0]).start(priority=s % 2)
        _loop(32, body)

    def w1_piece(p):
        idx = pl.ds(pl.multiple_of(p * 8, 8), 8)
        return pltpu.make_async_copy(w1_hbm.at[idx], w1_s.at[idx], w_sem.at[1])

    def w2_piece(p):
        idx = pl.ds(pl.multiple_of(p * 32, 32), 32)
        return pltpu.make_async_copy(w2_hbm.at[idx], w2_s.at[idx], w_sem.at[2])

    def start_ffn(half):
        def body(i):
            p = half * 14 + i
            w1_piece(p).start(priority=0)
            w2_piece(p).start(priority=1)
            w1_piece(32 + p).start(priority=0)
            w2_piece(28 + p).start(priority=1)
        _loop(14, body)
        if half == 1:
            def rest(i):
                w1_piece(28 + i).start(priority=0)
                w1_piece(60 + i).start(priority=1)
            _loop(4, rest)

    wo_base = [0]
    for runs in WO_PHASES:
        wo_base.append(wo_base[-1] + sum(n for _, n in runs) * DH)

    def start_wo(ph):
        runs = WO_PHASES[ph]
        rows = runs[0][1] * DH

        def body(i):
            for u, (h0, _) in enumerate(runs):
                src = pl.ds(pl.multiple_of(h0 * DH + i * 32, 32), 32)
                dst = pl.ds(pl.multiple_of(wo_base[ph] + u * rows + i * 32, 32), 32)
                pltpu.make_async_copy(wo_hbm.at[src], wo_s.at[dst], wo_sem.at[ph]).start(priority=u % 2)
        _loop(rows // 32, body)

    def start_kv(g, part):
        slot = g % NSLOT
        n = KV_PIECES // K_PARTS

        def body(i):
            idx = pl.ds(pl.multiple_of((part * n + i) * KV_ROWS, KV_ROWS), KV_ROWS)
            for b in (0, 2, 1, 3):
                pltpu.make_async_copy(k_hbm.at[b, g, idx], kv_s.at[slot, b, 0, idx],
                                      kv_sem.at[slot]).start(priority=0)
                pltpu.make_async_copy(v_hbm.at[b, g, idx], kv_s.at[slot, b, 1, idx],
                                      kv_sem.at[slot]).start(priority=1)
        _loop(n, body)

    def start_next(g, part):
        @pl.when(g + 1 < HKV)
        def _():
            start_kv(g + 1, part)

        @pl.when(g + 1 == HKV)
        def _():
            if part < 2:
                start_ffn(part)
            else:
                start_wo(part - 2)

    small[0].start()
    start_wq()
    for c in small[1:]:
        c.start()
    start_kv(0, 0)

    small[0].wait()
    xb = x_s[...]
    _wait_all(wq_s, w_sem.at[0])
    start_kv(0, 1)
    q = jnp.dot(xb, wq_s[...], preferred_element_type=jnp.float32)
    start_kv(0, 2)
    for h in range(HQ):
        q_s[h * 8:h * 8 + B, :] = q[:, h * DH:(h + 1) * DH]
    start_kv(0, 3)

    def attend(g, slot, b):
        rows = pl.ds(g * (REP * 8) + b, REP, stride=8)
        qv = q_s[rows, :].astype(jnp.bfloat16)
        s = lax.dot_general(qv, kv_s[slot, b, 0], _NT, preferred_element_type=jnp.float32) * SCALE
        m = jnp.max(s, axis=-1, keepdims=True)
        p = jnp.exp(s - m)
        l = jnp.sum(p, axis=-1, keepdims=True)
        o = jnp.dot(p.astype(jnp.bfloat16), kv_s[slot, b, 1], preferred_element_type=jnp.float32)
        o_s[rows, :] = o / l

    def group(g):
        slot = g % NSLOT
        start_next(g, 0)
        start_next(g, 1)
        _wait_all(kv_s.at[slot], kv_sem.at[slot])
        attend(g, slot, 0)
        start_next(g, 2)
        attend(g, slot, 1)
        start_next(g, 3)
        attend(g, slot, 2)
        attend(g, slot, 3)

    _loop(HKV, group)

    start_wo(2)
    small[2].wait()
    _wait_all(w1_s, w_sem.at[1])
    h1 = jnp.dot(xb, w1_s[...], preferred_element_type=jnp.float32)
    h1 = h1 + b1_s[...].astype(jnp.float32).reshape(1, F)
    r = jnp.maximum(h1, 0.0)
    hsq = (r * r).astype(jnp.bfloat16)
    small[3].wait()
    _wait_all(w2_s, w_sem.at[2])
    ffn = jnp.dot(hsq, w2_s[...], preferred_element_type=jnp.float32)
    ffn = ffn + b2_s[...].astype(jnp.float32).reshape(1, D)

    small[1].wait()
    xg = xb.astype(jnp.float32) * gw_s[...].astype(jnp.float32).reshape(1, D)
    gate = jax.nn.sigmoid(jnp.sum(xg, axis=-1, keepdims=True))
    ffn_part = (1.0 - gate) * ffn

    start_wo(3)
    attn = None
    for ph, runs in enumerate(WO_PHASES):
        _wait_all(wo_s.at[pl.ds(wo_base[ph], wo_base[ph + 1] - wo_base[ph])], wo_sem.at[ph])
        for u, (h0, n) in enumerate(runs):
            lhs = jnp.concatenate(
                [o_s[(h0 + j) * 8:(h0 + j) * 8 + B, :] for j in range(n)], axis=1).astype(jnp.bfloat16)
            r0 = wo_base[ph] + u * n * DH
            part = jnp.dot(lhs, wo_s[r0:r0 + n * DH, :], preferred_element_type=jnp.float32)
            attn = part if attn is None else attn + part

    o_ref[...] = (gate * attn + ffn_part).astype(o_ref.dtype)


@jax.jit
def pallas_gated_mix__gqa_block_cached__dense_activation_squared_relu__decode_kernel(
    A_x: jax.Array,
    A_k_cache: jax.Array,
    A_v_cache: jax.Array,
    A_wq: jax.Array,
    A_wo: jax.Array,
    B_x: jax.Array,
    B_w1: jax.Array,
    B_b1: jax.Array,
    B_w2: jax.Array,
    B_b2: jax.Array,
    gate_w: jax.Array,
):
    bf16 = jnp.bfloat16
    out = pl.pallas_call(
        _kernel,
        out_shape=jax.ShapeDtypeStruct((B, D), bf16),
        in_specs=[pl.BlockSpec(memory_space=_HBM)] * 10,
        out_specs=pl.BlockSpec(memory_space=pltpu.VMEM),
        scratch_shapes=[
            pltpu.VMEM((B, D), bf16),
            pltpu.VMEM((D,), bf16),
            pltpu.VMEM((F,), bf16),
            pltpu.VMEM((D,), bf16),
            pltpu.VMEM((D, HQ * DH), bf16),
            pltpu.VMEM((HQ * DH, D), bf16),
            pltpu.VMEM((D, F), bf16),
            pltpu.VMEM((F, D), bf16),
            pltpu.VMEM((NSLOT, B, 2, SK, DH), bf16),
            pltpu.VMEM((HQ * 8 + 8, DH), jnp.float32),
            pltpu.VMEM((HQ * 8 + 8, DH), jnp.float32),
            pltpu.SemaphoreType.DMA((4,)),
            pltpu.SemaphoreType.DMA((3,)),
            pltpu.SemaphoreType.DMA((len(WO_PHASES),)),
            pltpu.SemaphoreType.DMA((NSLOT,)),
        ],
        compiler_params=pltpu.CompilerParams(vmem_limit_bytes=64 * 1024 * 1024),
    )(A_x.reshape(B, D), A_k_cache, A_v_cache, A_wq, A_wo, B_w1, B_b1, B_w2, B_b2, gate_w)
    return out.reshape(B, 1, D)
```

```python
import functools

import jax
import jax.numpy as jnp
from jax import lax
import jax.experimental.pallas as pl
import jax.experimental.pallas.tpu as pltpu

B = 4
D = 512
HQ = 32
HKV = 8
REP = HQ // HKV
SK = 4096
DH = 128
F = 1792
SCALE = DH ** -0.5

KV_ROWS = 128
KV_PIECES = SK // KV_ROWS
K_PARTS = 4
NSLOT = 2

WO_PHASES = (
    tuple((4 * s, 2) for s in range(8)),
    tuple((4 * s + 2, 1) for s in range(8)),
    tuple((8 * s + 3, 1) for s in range(4)),
    tuple((8 * s + 7, 1) for s in range(4)),
)

_HBM = pltpu.MemorySpace.HBM
_NT = (((1,), (1,)), ((), ()))


def _loop(n, body):
    def step(i, carry):
        body(i)
        return carry
    lax.fori_loop(0, n, step, 0)


def _wait_all(buf, sem):
    pltpu.make_async_copy(buf, buf, sem).wait()


def _kernel(*refs):
    pl.run_scoped(
        functools.partial(_body, *refs),
        pltpu.SemaphoreType.DMA((4,)),
        pltpu.SemaphoreType.DMA((3,)),
        pltpu.SemaphoreType.DMA((len(WO_PHASES),)),
        pltpu.SemaphoreType.DMA((NSLOT,)),
    )


def _body(x_hbm, k_hbm, v_hbm, wq_hbm, wo_hbm, w1_hbm, b1_hbm, w2_hbm, b2_hbm, gw_hbm,
          o_ref,
          x_s, gw_s, b1_s, b2_s, wq_s, wo_s, w1_s, w2_s, kv_s, q_s, o_s,
          small_sem, w_sem, wo_sem, kv_sem):
    small = [
        pltpu.make_async_copy(x_hbm, x_s, small_sem.at[0]),
        pltpu.make_async_copy(gw_hbm, gw_s, small_sem.at[1]),
        pltpu.make_async_copy(b1_hbm, b1_s, small_sem.at[2]),
        pltpu.make_async_copy(b2_hbm, b2_s, small_sem.at[3]),
    ]

    def start_wq():
        def body(i):
            for s in range(4):
                p = s * 32 + i
                idx = (pl.ds(pl.multiple_of((p // 2) * 8, 8), 8),
                       pl.ds(pl.multiple_of((p % 2) * 2048, 2048), 2048))
                pltpu.make_async_copy(wq_hbm.at[idx], wq_s.at[idx], w_sem.at[0]).start(priority=s % 2)
        _loop(32, body)

    def w1_piece(p):
        idx = pl.ds(pl.multiple_of(p * 8, 8), 8)
        return pltpu.make_async_copy(w1_hbm.at[idx], w1_s.at[idx], w_sem.at[1])

    def w2_piece(p):
        idx = pl.ds(pl.multiple_of(p * 32, 32), 32)
        return pltpu.make_async_copy(w2_hbm.at[idx], w2_s.at[idx], w_sem.at[2])

    def start_ffn(half):
        def body(i):
            p = half * 14 + i
            w1_piece(p).start(priority=0)
            w2_piece(p).start(priority=1)
            w1_piece(32 + p).start(priority=0)
            w2_piece(28 + p).start(priority=1)
        _loop(14, body)
        if half == 1:
            def rest(i):
                w1_piece(28 + i).start(priority=0)
                w1_piece(60 + i).start(priority=1)
            _loop(4, rest)

    wo_base = [0]
    for runs in WO_PHASES:
        wo_base.append(wo_base[-1] + sum(n for _, n in runs) * DH)

    def start_wo(ph):
        runs = WO_PHASES[ph]
        rows = runs[0][1] * DH

        def body(i):
            for u, (h0, _) in enumerate(runs):
                src = pl.ds(pl.multiple_of(h0 * DH + i * 32, 32), 32)
                dst = pl.ds(pl.multiple_of(wo_base[ph] + u * rows + i * 32, 32), 32)
                pltpu.make_async_copy(wo_hbm.at[src], wo_s.at[dst], wo_sem.at[ph]).start(priority=u % 2)
        _loop(rows // 32, body)

    def start_kv(g, part):
        slot = g % NSLOT
        n = KV_PIECES // K_PARTS

        def body(i):
            idx = pl.ds(pl.multiple_of((part * n + i) * KV_ROWS, KV_ROWS), KV_ROWS)
            for b in (0, 2, 1, 3):
                pltpu.make_async_copy(k_hbm.at[b, g, idx], kv_s.at[slot, b, 0, idx],
                                      kv_sem.at[slot]).start(priority=0)
                pltpu.make_async_copy(v_hbm.at[b, g, idx], kv_s.at[slot, b, 1, idx],
                                      kv_sem.at[slot]).start(priority=1)
        _loop(n, body)

    def start_next(g, part):
        @pl.when(g + 1 < HKV)
        def _():
            start_kv(g + 1, part)

        @pl.when(g + 1 == HKV)
        def _():
            if part < 2:
                start_ffn(part)
            else:
                start_wo(part - 2)

    small[0].start()
    start_wq()
    for c in small[1:]:
        c.start()
    start_kv(0, 0)

    small[0].wait()
    xb = x_s[...]
    _wait_all(wq_s, w_sem.at[0])
    start_kv(0, 1)
    q = jnp.dot(xb, wq_s[...], preferred_element_type=jnp.float32)
    start_kv(0, 2)
    for h in range(HQ):
        q_s[h * 8:h * 8 + B, :] = q[:, h * DH:(h + 1) * DH]
    start_kv(0, 3)

    def attend(g, slot, b):
        rows = pl.ds(g * (REP * 8) + b, REP, stride=8)
        qv = q_s[rows, :].astype(jnp.bfloat16)
        s = lax.dot_general(qv, kv_s[slot, b, 0], _NT, preferred_element_type=jnp.float32) * SCALE
        m = jnp.max(s, axis=-1, keepdims=True)
        p = jnp.exp(s - m)
        l = jnp.sum(p, axis=-1, keepdims=True)
        o = jnp.dot(p.astype(jnp.bfloat16), kv_s[slot, b, 1], preferred_element_type=jnp.float32)
        o_s[rows, :] = o / l

    def group(g):
        slot = g % NSLOT
        start_next(g, 0)
        start_next(g, 1)
        _wait_all(kv_s.at[slot], kv_sem.at[slot])
        attend(g, slot, 0)
        start_next(g, 2)
        attend(g, slot, 1)
        start_next(g, 3)
        attend(g, slot, 2)
        attend(g, slot, 3)

    _loop(HKV, group)

    start_wo(2)
    small[2].wait()
    _wait_all(w1_s, w_sem.at[1])
    h1 = jnp.dot(xb, w1_s[...], preferred_element_type=jnp.float32)
    h1 = h1 + b1_s[...].astype(jnp.float32).reshape(1, F)
    r = jnp.maximum(h1, 0.0)
    hsq = (r * r).astype(jnp.bfloat16)
    small[3].wait()
    _wait_all(w2_s, w_sem.at[2])
    ffn = jnp.dot(hsq, w2_s[...], preferred_element_type=jnp.float32)
    ffn = ffn + b2_s[...].astype(jnp.float32).reshape(1, D)

    small[1].wait()
    xg = xb.astype(jnp.float32) * gw_s[...].astype(jnp.float32).reshape(1, D)
    gate = jax.nn.sigmoid(jnp.sum(xg, axis=-1, keepdims=True))
    ffn_part = (1.0 - gate) * ffn

    start_wo(3)
    attn = None
    for ph, runs in enumerate(WO_PHASES):
        _wait_all(wo_s.at[pl.ds(wo_base[ph], wo_base[ph + 1] - wo_base[ph])], wo_sem.at[ph])
        for u, (h0, n) in enumerate(runs):
            lhs = jnp.concatenate(
                [o_s[(h0 + j) * 8:(h0 + j) * 8 + B, :] for j in range(n)], axis=1).astype(jnp.bfloat16)
            r0 = wo_base[ph] + u * n * DH
            part = jnp.dot(lhs, wo_s[r0:r0 + n * DH, :], preferred_element_type=jnp.float32)
            attn = part if attn is None else attn + part

    o_ref[...] = (gate * attn + ffn_part).astype(o_ref.dtype)


@jax.jit
def pallas_gated_mix__gqa_block_cached__dense_activation_squared_relu__decode_kernel(
    A_x: jax.Array,
    A_k_cache: jax.Array,
    A_v_cache: jax.Array,
    A_wq: jax.Array,
    A_wo: jax.Array,
    B_x: jax.Array,
    B_w1: jax.Array,
    B_b1: jax.Array,
    B_w2: jax.Array,
    B_b2: jax.Array,
    gate_w: jax.Array,
):
    bf16 = jnp.bfloat16
    out = pl.pallas_call(
        _kernel,
        out_shape=jax.ShapeDtypeStruct((B, D), bf16),
        in_specs=[pl.BlockSpec(memory_space=_HBM)] * 10,
        out_specs=pl.BlockSpec(memory_space=pltpu.VMEM),
        scratch_shapes=[
            pltpu.VMEM((B, D), bf16),
            pltpu.VMEM((D,), bf16),
            pltpu.VMEM((F,), bf16),
            pltpu.VMEM((D,), bf16),
            pltpu.VMEM((D, HQ * DH), bf16),
            pltpu.VMEM((HQ * DH, D), bf16),
            pltpu.VMEM((D, F), bf16),
            pltpu.VMEM((F, D), bf16),
            pltpu.VMEM((NSLOT, B, 2, SK, DH), bf16),
            pltpu.VMEM((HQ * 8 + 8, DH), jnp.float32),
            pltpu.VMEM((HQ * 8 + 8, DH), jnp.float32),
        ],
        compiler_params=pltpu.CompilerParams(vmem_limit_bytes=64 * 1024 * 1024),
    )(A_x.reshape(B, D), A_k_cache, A_v_cache, A_wq, A_wo, B_w1, B_b1, B_w2, B_b2, gate_w)
    return out.reshape(B, 1, D)
```

```python
import functools

import jax
import jax.numpy as jnp
from jax import lax
import jax.experimental.pallas as pl
import jax.experimental.pallas.tpu as pltpu

B = 4
D = 512
HQ = 32
HKV = 8
REP = HQ // HKV
SK = 4096
DH = 128
F = 1792
SCALE = DH ** -0.5

KV_ROWS = 128
KV_PIECES = SK // KV_ROWS
K_PARTS = 4
NSLOT = 2

WO_PHASES = (
    tuple((4 * s, 2) for s in range(8)),
    tuple((4 * s + 2, 1) for s in range(8)),
    tuple((8 * s + 3, 1) for s in range(4)),
    tuple((8 * s + 7, 1) for s in range(4)),
)
WO_STARTS = ((0,), (), (1,), (2, 3))

_HBM = pltpu.MemorySpace.HBM
_NT = (((1,), (1,)), ((), ()))


def _loop(n, body):
    def step(i, carry):
        body(i)
        return carry
    lax.fori_loop(0, n, step, 0)


def _wait_all(buf, sem):
    pltpu.make_async_copy(buf, buf, sem).wait()


def _kernel(*refs):
    pl.run_scoped(
        functools.partial(_body, *refs),
        pltpu.SemaphoreType.DMA((4,)),
        pltpu.SemaphoreType.DMA((3,)),
        pltpu.SemaphoreType.DMA((len(WO_PHASES),)),
        pltpu.SemaphoreType.DMA((NSLOT,)),
    )


def _body(x_hbm, k_hbm, v_hbm, wq_hbm, wo_hbm, w1_hbm, b1_hbm, w2_hbm, b2_hbm, gw_hbm,
          o_ref,
          x_s, gw_s, b1_s, b2_s, wq_s, wo_s, w1_s, w2_s, kv_s, q_s, o_s,
          small_sem, w_sem, wo_sem, kv_sem):
    small = [
        pltpu.make_async_copy(x_hbm, x_s, small_sem.at[0]),
        pltpu.make_async_copy(gw_hbm, gw_s, small_sem.at[1]),
        pltpu.make_async_copy(b1_hbm, b1_s, small_sem.at[2]),
        pltpu.make_async_copy(b2_hbm, b2_s, small_sem.at[3]),
    ]

    def start_weights():
        def body(i):
            for s in range(4):
                p = s * 32 + i
                idx = (pl.ds(pl.multiple_of((p // 2) * 8, 8), 8),
                       pl.ds(pl.multiple_of((p % 2) * 2048, 2048), 2048))
                pltpu.make_async_copy(wq_hbm.at[idx], wq_s.at[idx], w_sem.at[0]).start(priority=0)
                if s % 2 == 0:
                    idx = pl.ds(pl.multiple_of(((s // 2) * 32 + i) * 8, 8), 8)
                    pltpu.make_async_copy(w1_hbm.at[idx], w1_s.at[idx], w_sem.at[1]).start(priority=1)
                else:
                    @pl.when(i < 28)
                    def _():
                        idx = pl.ds(pl.multiple_of(((s // 2) * 28 + i) * 32, 32), 32)
                        pltpu.make_async_copy(w2_hbm.at[idx], w2_s.at[idx], w_sem.at[2]).start(priority=1)
        _loop(32, body)

    wo_base = [0]
    for runs in WO_PHASES:
        wo_base.append(wo_base[-1] + sum(n for _, n in runs) * DH)

    def start_wo(ph):
        runs = WO_PHASES[ph]
        rows = runs[0][1] * DH

        def body(i):
            for u, (h0, _) in enumerate(runs):
                src = pl.ds(pl.multiple_of(h0 * DH + i * 32, 32), 32)
                dst = pl.ds(pl.multiple_of(wo_base[ph] + u * rows + i * 32, 32), 32)
                pltpu.make_async_copy(wo_hbm.at[src], wo_s.at[dst], wo_sem.at[ph]).start(priority=u % 2)
        _loop(rows // 32, body)

    def start_kv(g, part):
        slot = g % NSLOT
        n = KV_PIECES // K_PARTS

        def body(i):
            idx = pl.ds(pl.multiple_of((part * n + i) * KV_ROWS, KV_ROWS), KV_ROWS)
            for b in (0, 2, 1, 3):
                pltpu.make_async_copy(k_hbm.at[b, g, idx], kv_s.at[slot, b, 0, idx],
                                      kv_sem.at[slot]).start(priority=0)
                pltpu.make_async_copy(v_hbm.at[b, g, idx], kv_s.at[slot, b, 1, idx],
                                      kv_sem.at[slot]).start(priority=1)
        _loop(n, body)

    def start_next(g, part):
        @pl.when(g + 1 < HKV)
        def _():
            start_kv(g + 1, part)

        @pl.when(g + 1 == HKV)
        def _():
            for ph in WO_STARTS[part]:
                start_wo(ph)

    for c in small:
        c.start()
    start_weights()
    start_kv(0, 0)
    q_s[...] = jnp.zeros(q_s.shape, q_s.dtype)
    o_s[...] = jnp.zeros(o_s.shape, o_s.dtype)

    small[0].wait()
    xb = x_s[...]
    _wait_all(wq_s, w_sem.at[0])
    start_kv(0, 1)
    q = jnp.dot(xb, wq_s[...], preferred_element_type=jnp.float32)
    for h in range(HQ):
        q_s[h * 8:h * 8 + B, :] = q[:, h * DH:(h + 1) * DH]
    start_kv(0, 2)

    small[2].wait()
    _wait_all(w1_s, w_sem.at[1])
    h1 = jnp.dot(xb, w1_s[...], preferred_element_type=jnp.float32)
    h1 = h1 + b1_s[...].astype(jnp.float32).reshape(1, F)
    r = jnp.maximum(h1, 0.0)
    hsq = (r * r).astype(jnp.bfloat16)
    small[3].wait()
    _wait_all(w2_s, w_sem.at[2])
    ffn = jnp.dot(hsq, w2_s[...], preferred_element_type=jnp.float32)
    ffn = ffn + b2_s[...].astype(jnp.float32).reshape(1, D)

    small[1].wait()
    xg = xb.astype(jnp.float32) * gw_s[...].astype(jnp.float32).reshape(1, D)
    gate = jax.nn.sigmoid(jnp.sum(xg, axis=-1, keepdims=True))
    ffn_part = (1.0 - gate) * ffn
    start_kv(0, 3)

    def attend(g, slot, b):
        rows = pl.ds(g * (REP * 8) + b, REP, stride=8)
        qv = q_s[rows, :].astype(jnp.bfloat16)
        s = lax.dot_general(qv, kv_s[slot, b, 0], _NT, preferred_element_type=jnp.float32) * SCALE
        m = jnp.max(s, axis=-1, keepdims=True)
        p = jnp.exp(s - m)
        l = jnp.sum(p, axis=-1, keepdims=True)
        o = jnp.dot(p.astype(jnp.bfloat16), kv_s[slot, b, 1], preferred_element_type=jnp.float32)
        o_s[rows, :] = o / l

    def group(g):
        slot = g % NSLOT
        start_next(g, 0)
        start_next(g, 1)
        _wait_all(kv_s.at[slot], kv_sem.at[slot])
        attend(g, slot, 0)
        start_next(g, 2)
        attend(g, slot, 1)
        start_next(g, 3)
        attend(g, slot, 2)
        attend(g, slot, 3)

    _loop(HKV, group)

    attn = None
    for ph, runs in enumerate(WO_PHASES):
        _wait_all(wo_s.at[pl.ds(wo_base[ph], wo_base[ph + 1] - wo_base[ph])], wo_sem.at[ph])
        for u, (h0, n) in enumerate(runs):
            lhs = jnp.concatenate(
                [o_s[(h0 + j) * 8:(h0 + j) * 8 + B, :] for j in range(n)], axis=1).astype(jnp.bfloat16)
            r0 = wo_base[ph] + u * n * DH
            part = jnp.dot(lhs, wo_s[r0:r0 + n * DH, :], preferred_element_type=jnp.float32)
            attn = part if attn is None else attn + part

    o_ref[...] = (gate * attn + ffn_part).astype(o_ref.dtype)


@jax.jit
def pallas_gated_mix__gqa_block_cached__dense_activation_squared_relu__decode_kernel(
    A_x: jax.Array,
    A_k_cache: jax.Array,
    A_v_cache: jax.Array,
    A_wq: jax.Array,
    A_wo: jax.Array,
    B_x: jax.Array,
    B_w1: jax.Array,
    B_b1: jax.Array,
    B_w2: jax.Array,
    B_b2: jax.Array,
    gate_w: jax.Array,
):
    bf16 = jnp.bfloat16
    out = pl.pallas_call(
        _kernel,
        out_shape=jax.ShapeDtypeStruct((B, D), bf16),
        in_specs=[pl.BlockSpec(memory_space=_HBM)] * 10,
        out_specs=pl.BlockSpec(memory_space=pltpu.VMEM),
        scratch_shapes=[
            pltpu.VMEM((B, D), bf16),
            pltpu.VMEM((D,), bf16),
            pltpu.VMEM((F,), bf16),
            pltpu.VMEM((D,), bf16),
            pltpu.VMEM((D, HQ * DH), bf16),
            pltpu.VMEM((HQ * DH, D), bf16),
            pltpu.VMEM((D, F), bf16),
            pltpu.VMEM((F, D), bf16),
            pltpu.VMEM((NSLOT, B, 2, SK, DH), bf16),
            pltpu.VMEM((HQ * 8 + 8, DH), jnp.float32),
            pltpu.VMEM((HQ * 8 + 8, DH), jnp.float32),
        ],
        compiler_params=pltpu.CompilerParams(vmem_limit_bytes=64 * 1024 * 1024),
    )(A_x.reshape(B, D), A_k_cache, A_v_cache, A_wq, A_wo, B_w1, B_b1, B_w2, B_b2, gate_w)
    return out.reshape(B, 1, D)
```
